```python
import os as _os
_os.environ.setdefault("JAX_PLATFORMS", "cpu")
import jax
import jax.numpy as jnp

def _softmax(x, axis=-1):
    return jax.nn.softmax(x, axis=axis)
def _gelu(x):
    return jax.nn.gelu(x, approximate=True)
def _silu(x):
    return jax.nn.silu(x)
def _sigmoid(x):
    return jax.nn.sigmoid(x)
def _layernorm(x, axis=-1, eps=1e-5):
    m = jnp.mean(x, axis=axis, keepdims=True)
    v = jnp.var(x, axis=axis, keepdims=True)
    return (x - m) / jnp.sqrt(v + eps)
def _scatter_add(tgt, idx, src, axis=0):
    return tgt.at[idx].add(src)
def _segment_sum(src, seg, n):
    return jax.ops.segment_sum(src, seg, n)
class _Rng:
    def __init__(self, key):
        self._k = key
    def _next(self):
        self._k, sub = jax.random.split(self._k)
        return sub
    def normal(self, shape):
        return jax.random.normal(self._next(), shape, dtype=jnp.bfloat16)
    def randint(self, lo, hi, shape):
        return jax.random.randint(self._next(), shape, lo, hi, dtype=jnp.int32)
    def uniform(self, shape, lo=0.0, hi=1.0):
        return jax.random.uniform(self._next(), shape, jnp.bfloat16, lo, hi)
    def permutation(self, n):
        return jax.random.permutation(self._next(), n)


kernel_name = 'parallel_sum__ssm_conv_h3__dense_activation_silu__prompt'

def setup_inputs():
    _rng = _Rng(jax.random.key(int.from_bytes(__import__("os").urandom(4), "little")))
    _w = (lambda a: (lambda t: t.astype(jnp.bfloat16) if jnp.issubdtype(t.dtype, jnp.floating) else t)(jnp.asarray(a)))
    def _A_setup():
        B, S, D = 1, 2048, 448
        ks = 4
        return {
            "q": _w((lambda *s: _rng.normal(s) * 0.05)(B, S, D)),
            "k": _w((lambda *s: _rng.normal(s) * 0.2)(B, S, D)),
            "v": _w((lambda *s: _rng.normal(s) * 0.2)(B, S, D)),
            "shift_k": _w((lambda *s: _rng.normal(s) * 0.2)(D, ks) * 0.5),
            "ssm_k": _w((lambda *s: _rng.normal(s) * 0.2)(D, S) * (1.0 / S ** 0.5)),
            "ssm_D": _w((lambda *s: _rng.normal(s) * 0.2)(D)),
        }
    _A_in = _A_setup()

    def _B_setup():
        B, S, D, F = 1, 2048, 448, 1792
        return {
            "x": _w((lambda *s: _rng.normal(s) * 0.05)(B, S, D)),
            "w1": _w((lambda *s: _rng.normal(s) * 0.05)(D, F) * (D ** -0.5)),
            "w2": _w((lambda *s: _rng.normal(s) * 0.05)(F, D) * (F ** -0.5)),
        }
    _B_in = _B_setup()

    return {
        "A_q": _A_in["q"],
        "A_k": _A_in["k"],
        "A_v": _A_in["v"],
        "A_shift_k": _A_in["shift_k"],
        "A_ssm_k": _A_in["ssm_k"],
        "A_ssm_D": _A_in["ssm_D"],
        "B_x": _B_in["x"],
        "B_w1": _B_in["w1"],
        "B_w2": _B_in["w2"],
    }

def reference(A_q, A_k, A_v, A_shift_k, A_ssm_k, A_ssm_D, B_x, B_w1, B_w2):
    def _A_ref(q, k, v, shift_k, ssm_k, ssm_D):
        B, S, D = q.shape
        ks = shift_k.shape[-1]
        k_pad = jnp.pad(k, ((0, 0), (ks - 1, 0), (0, 0)))
        k_shift = jnp.zeros_like(k)
        for t in range(ks):
            k_shift = k_shift + k_pad[:, t:t + S, :] * shift_k[:, ks - 1 - t][None, None, :]
        kv = k_shift * v
        L = 2 * S
        kv_pad = jnp.pad(kv, ((0, 0), (0, S), (0, 0)))
        kf_pad = jnp.pad(ssm_k, ((0, 0), (0, S)))
        kv_f = (lambda x, axes=(-2,-1): jnp.fft.rfft2(x.astype(jnp.float32), axes=axes))(kv_pad[:, None, :, :], axes=(1, 2))
        kf_f = (lambda x, axes=(-2,-1): jnp.fft.rfft2(x.astype(jnp.float32), axes=axes))(kf_pad[:, None, :], axes=(1, 2))
        kf_f = (lambda x, *d: x.transpose(*d))(kf_f, 1, 2, 0)
        y_f = kv_f * kf_f[None, :, :, :]
        y = (lambda x, s, axes=(-2,-1): jnp.fft.irfft2(x, s=s, axes=axes).astype(jnp.bfloat16))(y_f, (1, L), axes=(1, 2))[:, 0, :S, :]
        y = y + kv * ssm_D[None, None, :]
        return q * y

    def _B_ref(x, w1, w2):
        h = jnp.einsum("bsd,df->bsf", x, w1)
        h = _silu(h)
        out = jnp.einsum("bsf,fd->bsd", h, w2)
        return out

    x = A_q
    xn = _layernorm(x, axis=-1)
    return x + _A_ref(xn, A_k, A_v, A_shift_k, A_ssm_k, A_ssm_D) + _B_ref(xn, B_w1, B_w2)
```

```python
import functools
import math

import jax
import jax.numpy as jnp
import jax.experimental.pallas as pl
import jax.experimental.pallas.tpu as pltpu

L = 128
R = 256
CH = 32


def _kernel(q_ref, k_ref, v_ref, sk_ref, ssm_ref, d_ref, w1_ref, w2_ref, o_ref,
            wf_s, winv_s, kext_s, win_s, uf_s, hf_s, yf_s, y_s):
    i = pl.program_id(0)
    nb = R // L
    D = q_ref.shape[-1]

    @pl.when(i == 0)
    def _init():
        f = jax.lax.broadcasted_iota(jnp.int32, (L, 2 * L), 0)
        n = jax.lax.broadcasted_iota(jnp.int32, (L, 2 * L), 1)
        m = ((2 * f + 1) * n) % (4 * L)
        ang = m.astype(jnp.float32) * (math.pi / (2 * L))
        wf_s[0:L, :] = jnp.cos(ang).astype(jnp.bfloat16)
        wf_s[L:2 * L, :] = (-jnp.sin(ang)).astype(jnp.bfloat16)
        n2 = jax.lax.broadcasted_iota(jnp.int32, (L, L), 0) + L
        f2 = jax.lax.broadcasted_iota(jnp.int32, (L, L), 1)
        m2 = ((2 * f2 + 1) * n2) % (4 * L)
        ang2 = m2.astype(jnp.float32) * (math.pi / (2 * L))
        winv_s[:, 0:L] = (jnp.cos(ang2) * (1.0 / L)).astype(jnp.bfloat16)
        winv_s[:, L:2 * L] = (jnp.sin(ang2) * (-1.0 / L)).astype(jnp.bfloat16)
        kext_s[0:8, :] = jnp.zeros((8, D), jnp.float32)
        win_s[0:L, :] = jnp.zeros((L, D), jnp.bfloat16)

    x = q_ref[...].astype(jnp.float32)
    mu = jnp.mean(x, axis=-1, keepdims=True)
    xc = x - mu
    var = jnp.mean(xc * xc, axis=-1, keepdims=True)
    xn = xc * jax.lax.rsqrt(var + 1e-5)
    xn_b = xn.astype(jnp.bfloat16)

    kf32 = k_ref[...].astype(jnp.float32)
    kext_s[8:8 + R, :] = kf32
    sk = sk_ref[...].astype(jnp.float32)
    ksh = kf32 * sk[0:1, :]
    for j in range(1, 4):
        ksh = ksh + kext_s[8 - j:8 - j + R, :] * sk[j:j + 1, :]
    kext_s[0:8, :] = kf32[R - 8:R, :]
    kv = ksh * v_ref[...].astype(jnp.float32)
    kv_b = kv.astype(jnp.bfloat16)

    for b in range(nb):
        a = i * nb + b
        win_s[L:2 * L, :] = kv_b[b * L:(b + 1) * L, :]
        uf_s[a] = jnp.dot(wf_s[...], win_s[...], preferred_element_type=jnp.float32)
        win_s[0:L, :] = kv_b[b * L:(b + 1) * L, :]
        hf_s[a] = jax.lax.dot_general(
            wf_s[:, 0:L], ssm_ref[:, b * L:(b + 1) * L],
            (((1,), (1,)), ((), ())), preferred_element_type=jnp.float32)
        for c in range(L // CH):
            r0 = c * CH

            def body(dl, carry):
                yr, yi = carry
                ur = uf_s[a - dl, r0:r0 + CH, :]
                ui = uf_s[a - dl, L + r0:L + r0 + CH, :]
                hr = hf_s[dl, r0:r0 + CH, :]
                hi = hf_s[dl, L + r0:L + r0 + CH, :]
                yr = yr + (ur * hr - ui * hi)
                yi = yi + (ur * hi + ui * hr)
                return yr, yi

            z = jnp.zeros((CH, D), jnp.float32)
            yr, yi = jax.lax.fori_loop(0, a + 1, body, (z, z))
            yf_s[r0:r0 + CH, :] = yr.astype(jnp.bfloat16)
            yf_s[L + r0:L + r0 + CH, :] = yi.astype(jnp.bfloat16)
        y_s[b * L:(b + 1) * L, :] = jnp.dot(
            winv_s[...], yf_s[...], preferred_element_type=jnp.float32)

    h = jnp.dot(xn_b, w1_ref[...], preferred_element_type=jnp.float32)
    h = h * jax.nn.sigmoid(h)
    ff = jnp.dot(h.astype(jnp.bfloat16), w2_ref[...], preferred_element_type=jnp.float32)

    y = y_s[...] + kv * d_ref[...].astype(jnp.float32)
    o_ref[...] = (x + xn * y + ff).astype(o_ref.dtype)


@jax.jit
def pallas_parallel_sum__ssm_conv_h3__dense_activation_silu__prompt_kernel(
    A_q, A_k, A_v, A_shift_k, A_ssm_k, A_ssm_D, B_x, B_w1, B_w2,
):
    B, S, D = A_q.shape
    F = B_w1.shape[1]
    q = A_q.reshape(S, D)
    k = A_k.reshape(S, D)
    v = A_v.reshape(S, D)
    sk = A_shift_k.T
    dd = A_ssm_D.reshape(1, D)
    nblk = S // L

    out = pl.pallas_call(
        _kernel,
        grid=(S // R,),
        in_specs=[
            pl.BlockSpec((R, D), lambda i: (i, 0)),
            pl.BlockSpec((R, D), lambda i: (i, 0)),
            pl.BlockSpec((R, D), lambda i: (i, 0)),
            pl.BlockSpec((4, D), lambda i: (0, 0)),
            pl.BlockSpec((D, R), lambda i: (0, i)),
            pl.BlockSpec((1, D), lambda i: (0, 0)),
            pl.BlockSpec((D, F), lambda i: (0, 0)),
            pl.BlockSpec((F, D), lambda i: (0, 0)),
        ],
        out_specs=pl.BlockSpec((R, D), lambda i: (i, 0)),
        out_shape=jax.ShapeDtypeStruct((S, D), A_q.dtype),
        scratch_shapes=[
            pltpu.VMEM((2 * L, 2 * L), jnp.bfloat16),
            pltpu.VMEM((L, 2 * L), jnp.bfloat16),
            pltpu.VMEM((8 + R, D), jnp.float32),
            pltpu.VMEM((2 * L, D), jnp.bfloat16),
            pltpu.VMEM((nblk, 2 * L, D), jnp.float32),
            pltpu.VMEM((nblk, 2 * L, D), jnp.float32),
            pltpu.VMEM((2 * L, D), jnp.bfloat16),
            pltpu.VMEM((R, D), jnp.float32),
        ],
        compiler_params=pltpu.CompilerParams(
            dimension_semantics=("arbitrary",),
            vmem_limit_bytes=64 * 1024 * 1024,
        ),
    )(q, k, v, sk, A_ssm_k, dd, B_w1, B_w2)
    return out.reshape(B, S, D)
```

```python
import math

import jax
import jax.numpy as jnp
import jax.experimental.pallas as pl
import jax.experimental.pallas.tpu as pltpu

L = 128
R = 256
CH = 64


def _kernel(q_ref, k_ref, v_ref, sk_ref, ssm_ref, d_ref, w1_ref, w2t_ref, o_ref,
            wf_s, winv_s, w1t_s, kext_s, win_s, uf_s, hf_s, yf_s, y_s):
    i = pl.program_id(0)
    nb = R // L
    D = q_ref.shape[0]

    @pl.when(i == 0)
    def _init():
        n = jax.lax.broadcasted_iota(jnp.int32, (2 * L, L), 0)
        f = jax.lax.broadcasted_iota(jnp.int32, (2 * L, L), 1)
        m = ((2 * f + 1) * n) % (4 * L)
        ang = m.astype(jnp.float32) * (math.pi / (2 * L))
        wf_s[:, 0:L] = jnp.cos(ang).astype(jnp.bfloat16)
        wf_s[:, L:2 * L] = (-jnp.sin(ang)).astype(jnp.bfloat16)
        f2 = jax.lax.broadcasted_iota(jnp.int32, (L, L), 0)
        n2 = jax.lax.broadcasted_iota(jnp.int32, (L, L), 1) + L
        m2 = ((2 * f2 + 1) * n2) % (4 * L)
        ang2 = m2.astype(jnp.float32) * (math.pi / (2 * L))
        winv_s[0:L, :] = (jnp.cos(ang2) * (1.0 / L)).astype(jnp.bfloat16)
        winv_s[L:2 * L, :] = (jnp.sin(ang2) * (-1.0 / L)).astype(jnp.bfloat16)
        kext_s[:, 0:128] = jnp.zeros((D, 128), jnp.float32)
        win_s[:, 0:L] = jnp.zeros((D, L), jnp.bfloat16)
        w1t_s[...] = w1_ref[...].astype(jnp.float32).T.astype(jnp.bfloat16)

    x = q_ref[...].astype(jnp.float32)
    mu = jnp.mean(x, axis=0, keepdims=True)
    xc = x - mu
    var = jnp.mean(xc * xc, axis=0, keepdims=True)
    xn = xc * jax.lax.rsqrt(var + 1e-5)
    xn_b = xn.astype(jnp.bfloat16)

    kf32 = k_ref[...].astype(jnp.float32)
    kext_s[:, 128:128 + R] = kf32
    sk = sk_ref[...].astype(jnp.float32)
    ksh = kf32 * sk[:, 0:1]
    for j in range(1, 4):
        ksh = ksh + pltpu.roll(kext_s[...], j, 1)[:, 128:128 + R] * sk[:, j:j + 1]
    kext_s[:, 0:128] = kf32[:, R - 128:R]
    kv = ksh * v_ref[...].astype(jnp.float32)
    kv_b = kv.astype(jnp.bfloat16)

    for b in range(nb):
        a = i * nb + b
        win_s[:, L:2 * L] = kv_b[:, b * L:(b + 1) * L]
        uf_s[a] = jnp.dot(win_s[...], wf_s[...], preferred_element_type=jnp.float32)
        win_s[:, 0:L] = kv_b[:, b * L:(b + 1) * L]
        hf_s[a] = jnp.dot(ssm_ref[:, b * L:(b + 1) * L], wf_s[0:L, :],
                          preferred_element_type=jnp.float32)
        for c in range(D // CH):
            r0 = c * CH

            def body(dl, carry):
                yr, yi = carry
                ur = uf_s[a - dl, r0:r0 + CH, 0:L]
                ui = uf_s[a - dl, r0:r0 + CH, L:2 * L]
                hr = hf_s[dl, r0:r0 + CH, 0:L]
                hi = hf_s[dl, r0:r0 + CH, L:2 * L]
                yr = yr + (ur * hr - ui * hi)
                yi = yi + (ur * hi + ui * hr)
                return yr, yi

            z = jnp.zeros((CH, L), jnp.float32)
            yr, yi = jax.lax.fori_loop(0, a + 1, body, (z, z))
            yf_s[r0:r0 + CH, 0:L] = yr.astype(jnp.bfloat16)
            yf_s[r0:r0 + CH, L:2 * L] = yi.astype(jnp.bfloat16)
        y_s[:, b * L:(b + 1) * L] = jnp.dot(
            yf_s[...], winv_s[...], preferred_element_type=jnp.float32)

    h = jnp.dot(w1t_s[...], xn_b, preferred_element_type=jnp.float32)
    h = h * jax.nn.sigmoid(h)
    ff = jnp.dot(w2t_ref[...], h.astype(jnp.bfloat16), preferred_element_type=jnp.float32)

    y = y_s[...] + kv * d_ref[...].astype(jnp.float32)
    o_ref[...] = (x + xn * y + ff).astype(o_ref.dtype)


@jax.jit
def pallas_parallel_sum__ssm_conv_h3__dense_activation_silu__prompt_kernel(
    A_q, A_k, A_v, A_shift_k, A_ssm_k, A_ssm_D, B_x, B_w1, B_w2,
):
    B, S, D = A_q.shape
    F = B_w1.shape[1]
    q = A_q.reshape(S, D).T
    k = A_k.reshape(S, D).T
    v = A_v.reshape(S, D).T
    dd = A_ssm_D.reshape(D, 1)
    w2t = B_w2.T
    nblk = S // L
    ks = A_shift_k.shape[1]

    out = pl.pallas_call(
        _kernel,
        grid=(S // R,),
        in_specs=[
            pl.BlockSpec((D, R), lambda i: (0, i)),
            pl.BlockSpec((D, R), lambda i: (0, i)),
            pl.BlockSpec((D, R), lambda i: (0, i)),
            pl.BlockSpec((D, ks), lambda i: (0, 0)),
            pl.BlockSpec((D, R), lambda i: (0, i)),
            pl.BlockSpec((D, 1), lambda i: (0, 0)),
            pl.BlockSpec((D, F), lambda i: (0, 0)),
            pl.BlockSpec((D, F), lambda i: (0, 0)),
        ],
        out_specs=pl.BlockSpec((D, R), lambda i: (0, i)),
        out_shape=jax.ShapeDtypeStruct((D, S), A_q.dtype),
        scratch_shapes=[
            pltpu.VMEM((2 * L, 2 * L), jnp.bfloat16),
            pltpu.VMEM((2 * L, L), jnp.bfloat16),
            pltpu.VMEM((F, D), jnp.bfloat16),
            pltpu.VMEM((D, 128 + R), jnp.float32),
            pltpu.VMEM((D, 2 * L), jnp.bfloat16),
            pltpu.VMEM((nblk, D, 2 * L), jnp.float32),
            pltpu.VMEM((nblk, D, 2 * L), jnp.float32),
            pltpu.VMEM((D, 2 * L), jnp.bfloat16),
            pltpu.VMEM((D, R), jnp.float32),
        ],
        compiler_params=pltpu.CompilerParams(
            dimension_semantics=("arbitrary",),
            vmem_limit_bytes=64 * 1024 * 1024,
        ),
    )(q, k, v, A_shift_k, A_ssm_k, dd, B_w1, w2t)
    return out.T.reshape(B, S, D)
```
